```python
import os as _os
_os.environ.setdefault("JAX_PLATFORMS", "cpu")
import jax
import jax.numpy as jnp

def _softmax(x, axis=-1):
    return jax.nn.softmax(x, axis=axis)
def _gelu(x):
    return jax.nn.gelu(x, approximate=True)
def _silu(x):
    return jax.nn.silu(x)
def _sigmoid(x):
    return jax.nn.sigmoid(x)
def _layernorm(x, axis=-1, eps=1e-5):
    m = jnp.mean(x, axis=axis, keepdims=True)
    v = jnp.var(x, axis=axis, keepdims=True)
    return (x - m) / jnp.sqrt(v + eps)
def _scatter_add(tgt, idx, src, axis=0):
    return tgt.at[idx].add(src)
def _segment_sum(src, seg, n):
    return jax.ops.segment_sum(src, seg, n)
class _Rng:
    def __init__(self, key):
        self._k = key
    def _next(self):
        self._k, sub = jax.random.split(self._k)
        return sub
    def normal(self, shape):
        return jax.random.normal(self._next(), shape, dtype=jnp.bfloat16)
    def randint(self, lo, hi, shape):
        return jax.random.randint(self._next(), shape, lo, hi, dtype=jnp.int32)
    def uniform(self, shape, lo=0.0, hi=1.0):
        return jax.random.uniform(self._next(), shape, jnp.bfloat16, lo, hi)
    def permutation(self, n):
        return jax.random.permutation(self._next(), n)


kernel_name = 'concat_heads__spectral_gfnet__mha_block__prompt'

def setup_inputs():
    _rng = _Rng(jax.random.key(int.from_bytes(__import__("os").urandom(4), "little")))
    _w = (lambda a: (lambda t: t.astype(jnp.bfloat16) if jnp.issubdtype(t.dtype, jnp.floating) else t)(jnp.asarray(a)))
    def _A_setup():
        B, S, D = 1, 2048, 576
        Df = D // 2 + 1
        return {
            "x": _w((lambda *s: _rng.normal(s) * 0.05)(B, S, D)),
            "w_r": _w((lambda *s: _rng.normal(s) * 0.05)(S, Df) * 0.02),
            "w_i": _w((lambda *s: _rng.normal(s) * 0.05)(S, Df) * 0.02),
        }
    _A_in = _A_setup()

    def _B_setup():
        B, S, D, H = 1, 2048, 576, 32
        return {
            "x": _w((lambda *s: _rng.normal(s) * 0.1)(B, S, D)),
            "wqkv": _w((lambda *s: _rng.normal(s) * 0.1)(D, 3 * D)),
            "wo": _w((lambda *s: _rng.normal(s) * 0.05)(D, D)),
        }
    _B_in = _B_setup()

    return {
        "A_x": _A_in["x"],
        "A_w_r": _A_in["w_r"],
        "A_w_i": _A_in["w_i"],
        "B_x": _B_in["x"],
        "B_wqkv": _B_in["wqkv"],
        "B_wo": _B_in["wo"],
    }

def reference(A_x, A_w_r, A_w_i, B_x, B_wqkv, B_wo):
    def _A_ref(x, w_r, w_i):
        B, S, D = x.shape
        X = (lambda x, axes=(-2,-1): jnp.fft.rfft2(x.astype(jnp.float32), axes=axes))(x, axes=(-2, -1))
        W = w_r + 1j * w_i
        X = X * W
        y = (lambda x, s, axes=(-2,-1): jnp.fft.irfft2(x, s=s, axes=axes).astype(jnp.bfloat16))(X, (S, D), axes=(-2, -1))
        return y

    def _B_ref(x, wqkv, wo):
        B, S, D = x.shape
        H = 32
        Dh = D // H
        qkv = (lambda x, *d: x.transpose(*d))((x @ wqkv).reshape(B, S, 3, H, Dh), 2, 0, 3, 1, 4)
        q, k, v = qkv[0], qkv[1], qkv[2]
        scores = jnp.einsum("bhqd,bhkd->bhqk", q, k) * (Dh ** -0.5)
        p = _softmax(scores, axis=-1)
        o = jnp.einsum("bhqk,bhkd->bhqd", p, v)
        return (lambda x, *d: x.transpose(*d))(o, 0, 2, 1, 3).reshape(B, S, D) @ wo

    a = _A_ref(A_x, A_w_r, A_w_i)
    b = _B_ref(B_x, B_wqkv, B_wo)
    return jnp.concatenate([a, b], axis=-1)
```

```python
import functools
import math

import numpy as np
import jax
import jax.numpy as jnp
import jax.experimental.pallas as pl
import jax.experimental.pallas.tpu as pltpu

S = 2048
D = 576
H = 32
DH = 18
DF = D // 2 + 1
NR = 296
HPG = 7
NG = 5
TQ = 512
TK = 256
NQ = S // TQ
NK = S // TK
GW = NG * 128
OP = 24
F32 = jnp.float32
BF16 = jnp.bfloat16

_C1 = math.cos(math.pi / 8)
_C3 = math.cos(3 * math.pi / 8)
_R2 = math.cos(math.pi / 4)


def _dft_constants():
    k2 = np.arange(DF)[:, None]
    m = np.arange(D)[None, :]
    fdm = np.zeros((2 * NR, D), np.float64)
    ang = 2 * np.pi * ((k2 * m) % D) / D
    fdm[:DF] = np.cos(ang)
    fdm[NR:NR + DF] = -np.sin(ang)
    n2 = np.arange(128)[:, None]
    j = np.arange(128)[None, :]
    g = np.zeros((16, 256, 256), np.float64)
    for k1 in range(16):
        a = -2 * np.pi * ((n2 * (k1 + 16 * j)) % S) / S
        cr, ci = np.cos(a), np.sin(a)
        g[k1] = np.block([[cr, ci], [-ci, cr]])
    return fdm.astype(np.float32), g.astype(np.float32)


_FDM_NP, _G_NP = _dft_constants()
_QSCALE = float(np.asarray(DH ** -0.5, np.float32).astype(jnp.bfloat16).astype(np.float32)) * math.log2(math.e)


def _rfft16(x):
    a = [x[n] + x[n + 8] for n in range(8)]
    b = [x[n] - x[n + 8] for n in range(8)]
    c = [a[n] + a[n + 4] for n in range(4)]
    d = [a[n] - a[n + 4] for n in range(4)]
    s02, s13 = c[0] + c[2], c[1] + c[3]
    x0, x8 = s02 + s13, s02 - s13
    x4r, x4i = c[0] - c[2], c[3] - c[1]
    t1 = (d[1] - d[3]) * _R2
    t2 = (d[1] + d[3]) * _R2
    x2r, x6r = d[0] + t1, d[0] - t1
    x2i, x6i = -(d[2] + t2), d[2] - t2
    e = {n: b[n] - b[8 - n] for n in (1, 2, 3)}
    f = {n: b[n] + b[8 - n] for n in (1, 2, 3)}
    re2 = e[2] * _R2
    u, v = b[0] + re2, b[0] - re2
    p = e[1] * _C1 + e[3] * _C3
    s = e[1] * _C3 - e[3] * _C1
    x1r, x7r, x3r, x5r = u + p, u - p, v + s, v - s
    g = f[2] * _R2
    pp = f[1] * _C3 + f[3] * _C1
    qq = f[1] * _C1 - f[3] * _C3
    g1, g2 = g + b[4], g - b[4]
    x1i, x7i = -(pp + g1), g1 - pp
    x3i, x5i = -(qq + g2), g2 - qq
    return [x0, x8, x1r, x1i, x2r, x2i, x3r, x3i, x4r, x4i, x5r, x5i, x6r, x6i, x7r, x7i]


def _irfft16(h):
    h0, h8, h1r, h1i, h2r, h2i, h3r, h3i, h4r, h4i, h5r, h5i, h6r, h6i, h7r, h7i = h
    u, pp = h1r + h7r, h1r - h7r
    v, ss = h3r + h5r, h3r - h5r
    b0 = u + v
    e2 = (u - v) * _R2
    e1 = pp * _C1 + ss * _C3
    e3 = pp * _C3 - ss * _C1
    p1, g1 = -(h1i + h7i), h7i - h1i
    q1, g2 = -(h3i + h5i), h5i - h3i
    b4 = g1 - g2
    f2 = (g1 + g2) * _R2
    f1 = p1 * _C3 + q1 * _C1
    f3 = p1 * _C1 - q1 * _C3
    b = [b0, e1 + f1, e2 + f2, e3 + f3, b4, f3 - e3, f2 - e2, f1 - e1]
    d0 = h2r + h6r
    t1 = (h2r - h6r) * _R2
    d2 = h6i - h2i
    t2 = (h2i + h6i) * (-_R2)
    d = [d0, t1 + t2, d2, t2 - t1]
    s02, s13 = h0 + h8, h0 - h8
    c = [s02 + h4r, s13 - h4i, s02 - h4r, s13 + h4i]
    a = [c[n] + d[n] for n in range(4)] + [c[n] - d[n] for n in range(4)]
    return [a[n] + b[n] for n in range(8)] + [a[n] - b[n] for n in range(8)]


def _dot(a, b, dims):
    return jax.lax.dot_general(a, b, (dims, ((), ())), preferred_element_type=F32)


_NN = ((1,), (0,))
_NT = ((1,), (1,))
_TN = ((0,), (0,))
_TT = ((0,), (1,))


def _kernel(ax_hbm, wr_hbm, wi_hbm, bx_hbm, wqkv_hbm, wo_hbm, fdm_hbm, g_hbm,
            out_hbm,
            ax_ref, wr_ref, wi_ref, bx_ref, wqkv_ref, wo_ref, fdm_ref, g_ref,
            out_ref, wt32_ref, wt_ref, wtail_ref, wop_ref, wop32_ref, k_ref, qt_ref, vt32_ref, vtp_ref, vt_ref, ot_ref,
            s0_ref, s1_ref, m_ref, r_ref, hh_ref, wr32_ref, wi32_ref,
            in_sems, out_sems):
    qscale = _QSCALE

    srcs = (bx_hbm, wqkv_hbm, ax_hbm, fdm_hbm, wr_hbm, wi_hbm, g_hbm, wo_hbm)
    dsts = (bx_ref, wqkv_ref, ax_ref, fdm_ref, wr_ref, wi_ref, g_ref, wo_ref)
    copies = [pltpu.make_async_copy(s, d, in_sems.at[i]) for i, (s, d) in enumerate(zip(srcs, dsts))]
    for cp in copies:
        cp.start()
    cp_bx, cp_wqkv, cp_ax, cp_fdm, cp_wr, cp_wi, cp_g, cp_wo = copies

    cp_wqkv.wait()
    with jax.named_scope("wprep"):
        wt32_ref[...] = jnp.zeros(wt32_ref.shape, F32)
        for t in range(3):
            wt = wqkv_ref[:, t * D:(t + 1) * D].astype(F32).T
            if t == 2:
                wt32_ref[2 * GW:2 * GW + D, :] = wt
            else:
                for g in range(NG):
                    w = min(HPG, H - g * HPG) * DH
                    r0 = g * HPG * DH
                    wt32_ref[t * GW + g * 128:t * GW + g * 128 + w, :] = wt[r0:r0 + w, :]
        wt_ref[...] = wt32_ref[...].astype(BF16)
    cp_bx.wait()

    PC = 512

    def proj_body(i, _):
        c0 = pl.multiple_of(i * PC, PC)
        pr = _dot(wt_ref[...], bx_ref[:, pl.ds(c0, PC)], _NN)
        for g in range(NG):
            qt_ref[g, :, pl.ds(c0, PC)] = pr[g * 128:(g + 1) * 128, :] * qscale
            k_ref[g, pl.ds(c0, PC), :] = pr[GW + g * 128:GW + (g + 1) * 128, :].astype(BF16).T
        vt32_ref[:, pl.ds(c0, PC)] = pr[2 * GW:, :]
        return 0

    with jax.named_scope("proj"):
        jax.lax.fori_loop(0, S // PC, proj_body, 0)

    with jax.named_scope("vprep"):
        rows32 = jax.lax.broadcasted_iota(jnp.int32, (32, S), 0)
        vtp_ref[...] = jnp.where(rows32 == DH, 1.0, 0.0).astype(F32)
        for h in range(H):
            vtp_ref[0:DH, :] = vt32_ref[h * DH:(h + 1) * DH, :]
            vt_ref[h] = vtp_ref[...].astype(BF16)

    cp_ax.wait()
    RC = 64

    def fwd16_body(i, _):
        r0 = pl.multiple_of(i * RC, RC)
        xs = [ax_ref[pl.ds(r0, RC), a * 128:(a + 1) * 128].astype(F32) for a in range(16)]
        ys = _rfft16(xs)
        for b in range(16):
            r_ref[b, pl.ds(r0, RC), :] = ys[b].astype(BF16)
        return 0

    with jax.named_scope("fwd16"):
        jax.lax.fori_loop(0, D // RC, fwd16_body, 0)

    cp_wr.wait()
    cp_wi.wait()
    with jax.named_scope("filtprep"):
        for src, dst in ((wr_ref, wr32_ref), (wi_ref, wi32_ref)):
            dst[0] = src[0:128, :].astype(F32).T
            dst[1] = src[128:256, :].astype(F32).T
            wtail_ref[...] = jnp.zeros(wtail_ref.shape, F32)
            wtail_ref[0:DF - 256, :] = src[256:DF, :].astype(F32)
            dst[2] = wtail_ref[...].T
    cp_fdm.wait()
    cp_g.wait()

    frow = jax.lax.broadcasted_iota(jnp.int32, (NR, 128), 0)
    cfac = jnp.where((frow == 0) | (frow == DF - 1), 1.0, 2.0).astype(F32) * (1.0 / (S * D))

    def filt_t(w_ref, k1):
        parts = [w_ref[t, pl.ds(k1, 128, stride=16), :].T for t in range(3)]
        parts[2] = parts[2][:NR - 256]
        return jnp.concatenate(parts, axis=0) * cfac

    def spectral(k1, lr, li):
        gm = g_ref[k1]
        y = _dot(jnp.concatenate([lr, li], axis=1).astype(BF16), gm, _NN)
        yr, yi = y[:, :128], y[:, 128:]
        wr = filt_t(wr32_ref, k1)
        wi = filt_t(wi32_ref, k1)
        z = jnp.concatenate([yr * wr - yi * wi, yr * wi + yi * wr], axis=1).astype(BF16)
        b = _dot(z, gm, _NT)
        return b[:, :128], b[:, 128:]

    def fwd_d(blk):
        t = _dot(fdm_ref[...], blk, _NN)
        return t[:NR], t[NR:]

    def inv_d(ur, ui):
        u = jnp.concatenate([ur, ui], axis=0).astype(BF16)
        return _dot(u, fdm_ref[...], _TN)

    def pair_body(k1, _):
        drr, dir_ = fwd_d(r_ref[2 * k1])
        dri, dii = fwd_d(r_ref[2 * k1 + 1])
        br1, bi1 = spectral(k1, drr - dii, dir_ + dri)
        br2, bi2 = spectral(16 - k1, drr + dii, dir_ - dri)
        hh_ref[2 * k1] = inv_d(br1 + br2, bi1 + bi2)
        hh_ref[2 * k1 + 1] = inv_d(bi1 - bi2, br2 - br1)
        return 0

    with jax.named_scope("spectral"):
        for p, k1 in ((0, 0), (1, 8)):
            lr, li = fwd_d(r_ref[p])
            br, bi = spectral(k1, lr, li)
            hh_ref[p] = inv_d(br, bi)
        jax.lax.fori_loop(1, 8, pair_body, 0)

    IC = 16

    def inv16_body(i, _):
        r0 = pl.multiple_of(i * IC, IC)
        hs = [hh_ref[b, pl.ds(r0, IC), :] for b in range(16)]
        ys = _irfft16(hs)
        for a in range(16):
            out_ref[pl.ds(a * 128 + r0, IC), 0:D] = ys[a].astype(BF16)
        return 0

    with jax.named_scope("inv16"):
        jax.lax.fori_loop(0, 128 // IC, inv16_body, 0)

    T = H * NQ
    qrows = jax.lax.broadcasted_iota(jnp.int32, (128, TQ), 0)

    def get_q(t):
        h = t // NQ
        j = t % NQ
        g = h // HPG
        lo = (h % HPG) * DH
        q = qt_ref[g, :, pl.ds(pl.multiple_of(j * TQ, TQ), TQ)]
        q = jnp.where((qrows >= lo) & (qrows < lo + DH), q, 0.0).astype(BF16)
        return g, q

    def stage_a(c, g, q, s_ref, m):
        s = _dot(k_ref[g, c * TK:(c + 1) * TK, :], q, _NN)
        s_ref[c * TK:(c + 1) * TK, :] = s
        return jnp.maximum(m, jnp.max(s.reshape(TK // 8, 8, TQ), axis=0))

    def stage_b(c, h, s_ref, m, acc):
        p = jnp.exp2(s_ref[c * TK:(c + 1) * TK, :] - m).astype(BF16)
        return acc + _dot(vt_ref[h, :, c * TK:(c + 1) * TK], p, _NN)

    g0, q0 = get_q(0)
    m0 = jnp.full((8, TQ), -jnp.inf, F32)
    for c in range(NK):
        m0 = stage_a(c, g0, q0, s0_ref, m0)
    m_ref[...] = jnp.max(m0, axis=0, keepdims=True)

    def half(t, scur, snext):
        h = t // NQ
        j = t % NQ
        g, q = get_q(jnp.minimum(t + 1, T - 1))
        mcur = m_ref[...]
        mn = jnp.full((8, TQ), -jnp.inf, F32)
        acc = jnp.zeros((32, TQ), F32)
        for c in range(NK):
            mn = stage_a(c, g, q, snext, mn)
            acc = stage_b(c, h, scur, mcur, acc)
        m_ref[...] = jnp.max(mn, axis=0, keepdims=True)
        ot_ref[h, :, pl.ds(pl.multiple_of(j * TQ, TQ), TQ)] = acc[:OP] / acc[DH:DH + 1, :]

    def att_body(i, _):
        half(2 * i, s0_ref, s1_ref)
        half(2 * i + 1, s1_ref, s0_ref)
        return 0

    with jax.named_scope("attn"):
        jax.lax.fori_loop(0, T // 2, att_body, 0)

    cp_wo.wait()
    wop32_ref[...] = jnp.zeros(wop32_ref.shape, F32)
    wo32 = wo_ref[...].astype(F32)
    for h in range(H):
        wop32_ref[h * OP:h * OP + DH, :] = wo32[h * DH:(h + 1) * DH, :]
    wop_ref[...] = wop32_ref[...].astype(BF16)

    OC = 256
    NOC = S // OC

    def out_copy(i):
        r0 = pl.multiple_of(i * OC, OC)
        return pltpu.make_async_copy(out_ref.at[pl.ds(r0, OC), :], out_hbm.at[pl.ds(r0, OC), :],
                                     out_sems.at[i])

    def oproj_body(i, _):
        r0 = pl.multiple_of(i * OC, OC)
        o = ot_ref[:, :, pl.ds(r0, OC)].reshape(H * OP, OC).astype(BF16)
        out_ref[pl.ds(r0, OC), D:2 * D] = _dot(o, wop_ref[...], _TN).astype(BF16)
        out_copy(i).start()
        return 0

    with jax.named_scope("oproj"):
        jax.lax.fori_loop(0, NOC, oproj_body, 0)
    for i in range(NOC):
        out_copy(i).wait()


@jax.jit
def pallas_concat_heads__spectral_gfnet__mha_block__prompt_kernel(
    A_x: jax.Array,
    A_w_r: jax.Array,
    A_w_i: jax.Array,
    B_x: jax.Array,
    B_wqkv: jax.Array,
    B_wo: jax.Array,
):
    fdm = jnp.asarray(_FDM_NP, dtype=BF16)
    gm = jnp.asarray(_G_NP, dtype=BF16)
    any_spec = pl.BlockSpec(memory_space=pltpu.HBM)
    vm = pltpu.VMEM
    out = pl.pallas_call(
        _kernel,
        in_specs=[any_spec] * 8,
        out_specs=any_spec,
        out_shape=jax.ShapeDtypeStruct((S, 2 * D), BF16),
        scratch_shapes=[
            vm((D, S), BF16), vm((DF, S), BF16), vm((DF, S), BF16), vm((D, S), BF16),
            vm((D, 3 * D), BF16), vm((D, D), BF16), vm((2 * NR, D), BF16), vm((16, 256, 256), BF16),
            vm((S, 2 * D), BF16),
            vm((2 * GW + D, D), F32),
            vm((2 * GW + D, D), BF16),
            vm((128, S), F32),
            vm((H * OP, D), BF16),
            vm((H * OP, D), F32),
            vm((NG, S, 128), BF16),
            vm((NG, 128, S), F32),
            vm((D, S), F32),
            vm((32, S), F32),
            vm((H, 32, S), BF16),
            vm((H, OP, S), F32),
            vm((S, TQ), F32), vm((S, TQ), F32), vm((1, TQ), F32),
            vm((16, D, 128), BF16),
            vm((16, 128, D), F32),
            vm((3, S, 128), F32), vm((3, S, 128), F32),
            pltpu.SemaphoreType.DMA((8,)),
            pltpu.SemaphoreType.DMA((S // 256,)),
        ],
        compiler_params=pltpu.CompilerParams(vmem_limit_bytes=110 * 2 ** 20),
    )(A_x.reshape(S, D).T, A_w_r.T, A_w_i.T, B_x.reshape(S, D).T, B_wqkv, B_wo, fdm, gm)
    return out.reshape(1, S, 2 * D)
```

```python
import math

import numpy as np
import jax
import jax.numpy as jnp
import jax.experimental.pallas as pl
import jax.experimental.pallas.tpu as pltpu

S = 2048
D = 576
H = 32
DH = 18
DF = D // 2 + 1
NR = 296
HB = 16
_GS = (0, 6, 11)
NG = 6
TQ = 512
TK = 128
SKEW = 2
HPI = 2
PR = 40
NQ = S // TQ
NK = S // TK
OP = 24
F32 = jnp.float32
BF16 = jnp.bfloat16

_C1 = math.cos(math.pi / 8)
_C3 = math.cos(3 * math.pi / 8)
_R2 = math.cos(math.pi / 4)
_N1, _N2, _N4 = (math.cos(2 * math.pi * k / 9) for k in (1, 2, 4))
_S1, _S3, _S4 = (math.sin(2 * math.pi * k / 9) for k in (1, 3, 4))


def _dft_constants():
    b = np.arange(64)[None, :]
    f0 = np.zeros((128, 128))
    j = np.arange(33)[:, None]
    th = 2 * np.pi * ((b * 9 * j) % D) / D
    f0[:33, :64] = np.cos(th)
    f0[40:73, :64] = -np.sin(th)
    fc = np.zeros((5, 128, 128))
    fc[0] = f0
    j = np.arange(32)[:, None]
    for c in range(1, 5):
        th = 2 * np.pi * ((b * (c + 9 * j)) % D) / D
        th2 = 2 * np.pi * ((b * (9 - c + 9 * j)) % D) / D
        fc[c, 0:32] = np.concatenate([np.cos(th), np.sin(th)], 1)
        fc[c, 32:64] = np.concatenate([np.cos(th2), -np.sin(th2)], 1)
        fc[c, 64:96] = np.concatenate([-np.sin(th), np.cos(th)], 1)
        fc[c, 96:128] = np.concatenate([-np.sin(th2), -np.cos(th2)], 1)
    fd = np.concatenate([fc, fc.transpose(0, 2, 1)], 0)
    n2 = np.arange(128)[:, None]
    j = np.arange(128)[None, :]
    g = np.zeros((16, 256, 256))
    for k1 in range(16):
        a = -2 * np.pi * ((n2 * (k1 + 16 * j)) % S) / S
        cr, ci = np.cos(a), np.sin(a)
        g[k1] = np.block([[cr, ci], [-ci, cr]])
    return fd.astype(np.float32), g.astype(np.float32)


_FD_NP, _G_NP = _dft_constants()
_QSCALE = float(np.asarray(DH ** -0.5, np.float32).astype(jnp.bfloat16).astype(np.float32)) * math.log2(math.e)
_RES = [(0, 33, 0)] + [r for c in range(1, 5)
                       for r in ((c, 32, 40 + 64 * (c - 1)), (9 - c, 32, 72 + 64 * (c - 1)))]


def _rfft16(x):
    a = [x[n] + x[n + 8] for n in range(8)]
    b = [x[n] - x[n + 8] for n in range(8)]
    c = [a[n] + a[n + 4] for n in range(4)]
    d = [a[n] - a[n + 4] for n in range(4)]
    s02, s13 = c[0] + c[2], c[1] + c[3]
    x0, x8 = s02 + s13, s02 - s13
    x4r, x4i = c[0] - c[2], c[3] - c[1]
    t1 = (d[1] - d[3]) * _R2
    t2 = (d[1] + d[3]) * _R2
    x2r, x6r = d[0] + t1, d[0] - t1
    x2i, x6i = -(d[2] + t2), d[2] - t2
    e = {n: b[n] - b[8 - n] for n in (1, 2, 3)}
    f = {n: b[n] + b[8 - n] for n in (1, 2, 3)}
    re2 = e[2] * _R2
    u, v = b[0] + re2, b[0] - re2
    p = e[1] * _C1 + e[3] * _C3
    s = e[1] * _C3 - e[3] * _C1
    x1r, x7r, x3r, x5r = u + p, u - p, v + s, v - s
    g = f[2] * _R2
    pp = f[1] * _C3 + f[3] * _C1
    qq = f[1] * _C1 - f[3] * _C3
    g1, g2 = g + b[4], g - b[4]
    x1i, x7i = -(pp + g1), g1 - pp
    x3i, x5i = -(qq + g2), g2 - qq
    return [x0, x8, x1r, x1i, x2r, x2i, x3r, x3i, x4r, x4i, x5r, x5i, x6r, x6i, x7r, x7i]


def _irfft16(h):
    h0, h8, h1r, h1i, h2r, h2i, h3r, h3i, h4r, h4i, h5r, h5i, h6r, h6i, h7r, h7i = h
    u, pp = h1r + h7r, h1r - h7r
    v, ss = h3r + h5r, h3r - h5r
    b0 = u + v
    e2 = (u - v) * _R2
    e1 = pp * _C1 + ss * _C3
    e3 = pp * _C3 - ss * _C1
    p1, g1 = -(h1i + h7i), h7i - h1i
    q1, g2 = -(h3i + h5i), h5i - h3i
    b4 = g1 - g2
    f2 = (g1 + g2) * _R2
    f1 = p1 * _C3 + q1 * _C1
    f3 = p1 * _C1 - q1 * _C3
    b = [b0, e1 + f1, e2 + f2, e3 + f3, b4, f3 - e3, f2 - e2, f1 - e1]
    d0 = h2r + h6r
    t1 = (h2r - h6r) * _R2
    d2 = h6i - h2i
    t2 = (h2i + h6i) * (-_R2)
    d = [d0, t1 + t2, d2, t2 - t1]
    s02, s13 = h0 + h8, h0 - h8
    c = [s02 + h4r, s13 - h4i, s02 - h4r, s13 + h4i]
    a = [c[n] + d[n] for n in range(4)] + [c[n] - d[n] for n in range(4)]
    return [a[n] + b[n] for n in range(8)] + [a[n] - b[n] for n in range(8)]


def _rfft9(x):
    s1, s2, s3, s4 = [x[a] + x[9 - a] for a in (1, 2, 3, 4)]
    d1, d2, d3, d4 = [x[a] - x[9 - a] for a in (1, 2, 3, 4)]
    t = x[0] - 0.5 * s3
    u = s1 + s2 + s4
    z = x[0] + s3
    a0 = z + u
    ar3 = z - 0.5 * u
    p, q = s1 - s4, s2 - s4
    ar1 = t + (_N1 * p + _N2 * q)
    ar2 = t + (_N2 * p + _N4 * q)
    ar4 = t + (_N4 * p + _N1 * q)
    e, f, g = d1 + d2, d2 + d4, d1 - d4
    w = _S3 * d3
    ai1 = ((-_S1) * e - _S4 * f) - w
    ai2 = w - (_S1 * g + _S4 * e)
    ai4 = (_S1 * f - _S4 * g) - w
    ai3 = (d2 - d1 - d4) * _S3
    return [a0, ar1, ai1, ar2, ai2, ar3, ai3, ar4, ai4]


def _irfft9(h):
    h0, hr1, hi1, hr2, hi2, hr3, hi3, hr4, hi4 = h
    t = hr1 + hr2 + hr4
    p = _N1 * (hr1 - hr4) + _N2 * (hr2 - hr4)
    q = _N2 * (hr1 - hr2) + _N1 * (hr4 - hr2)
    z = h0 + hr3
    u = h0 - 0.5 * hr3
    x0 = z + t
    s3 = z - 0.5 * t
    s1, s2, s4 = u + p, u + q, u - p - q
    e = (-_S1) * hi1 - _S4 * hi2
    f = _S1 * hi4 - _S4 * hi1
    g = (-_S1) * hi2 - _S4 * hi4
    d3 = (hi2 - hi1 - hi4) * _S3
    v = (-_S3) * hi3
    d1, d2, d4 = e + g + v, e + f - v, f - g + v
    return [x0, s1 + d1, s2 + d2, s3 + d3, s4 + d4, s4 - d4, s3 - d3, s2 - d2, s1 - d1]


def _dot(a, b, dims):
    return jax.lax.dot_general(a, b, (dims, ((), ())), preferred_element_type=F32)


_NN = ((1,), (0,))
_NT = ((1,), (1,))


def _kernel(ax_hbm, wr_hbm, wi_hbm, bx_hbm, wqkv_hbm, wo_hbm, fd_hbm, g_hbm,
            out_hbm,
            ax_ref, wr_ref, wi_ref, bx_ref, wqkv_ref, wo_ref, fd_ref, g_ref,
            out_ref, wt_ref, wot_ref, k_ref, kt_ref, qt_ref, vt_ref, ot_ref, wop_ref,
            s0_ref, s1_ref, m0_ref, m1_ref,
            u_ref, r_ref, t_ref, ub_ref, wa_ref, wb_ref, wc_ref, wf_ref,
            in_sems, out_sems):
    PC = 512
    NPC = S // PC
    wrs = [slice(0, 256), slice(256, 512), slice(512, D)]
    cp_w = [pltpu.make_async_copy(wqkv_hbm.at[rs, :], wqkv_ref.at[rs, :], in_sems.at[t])
            for t, rs in enumerate(wrs)]
    cp_bx = [pltpu.make_async_copy(bx_hbm.at[:, i * PC:(i + 1) * PC], bx_ref.at[:, i * PC:(i + 1) * PC],
                                   in_sems.at[3 + i]) for i in range(NPC)]
    srcs = (ax_hbm, wr_hbm, wi_hbm, fd_hbm, g_hbm, wo_hbm)
    dsts = (ax_ref, wr_ref, wi_ref, fd_ref, g_ref, wo_ref)
    rest = [pltpu.make_async_copy(s, d, in_sems.at[3 + NPC + i]) for i, (s, d) in enumerate(zip(srcs, dsts))]
    cp_ax, cp_wr, cp_wi, cp_fd, cp_g, cp_wo = rest
    for cp in cp_w + cp_bx[:2] + rest[:3] + cp_bx[2:] + rest[3:]:
        cp.start()

    gws = [((_GS + (HB,))[gi + 1] - h0) * DH for gi, h0 in enumerate(_GS)]
    for g in range(NG):
        lo8 = gws[g % 3] // 8 * 8
        kt_ref[g, lo8:128, :] = jnp.zeros((128 - lo8, S), F32)

    def consts():
        for g in range(NG):
            lo8 = gws[g % 3] // 8 * 8
            qt_ref[g, lo8:128, :] = jnp.zeros((128 - lo8, S), F32)
        rows8 = jax.lax.broadcasted_iota(jnp.int32, (8, S), 0)
        tail = jnp.where(rows8 == DH - 16, 1.0, 0.0).astype(F32)
        for h in range(H):
            vt_ref[h, 16:OP, :] = tail
        ot_ref[:, 32:PR, :] = jnp.zeros((H // HPI, 8, S), F32)
        wb_ref[:, 32:40, :] = jnp.zeros((16, 8, 128), F32)
        wb_ref[:, NR:384, :] = jnp.zeros((16, 384 - NR, 128), F32)

    consts()

    for t in range(3):
        cp_w[t].wait()
        wt_ref[:, wrs[t]] = wqkv_ref[wrs[t], :].T

    def fwd9():
        for i in range(4):
            for qd in range(16):
                cs = slice(qd * 128, (qd + 1) * 128)
                xs = [ax_ref[a * 64 + i * 16:a * 64 + (i + 1) * 16, cs].astype(F32) for a in range(9)]
                ys = _rfft9(xs)
                for a in range(9):
                    u_ref[a * 64 + i * 16:a * 64 + (i + 1) * 16, cs] = ys[a]
                if qd % 4 == 3:
                    yield

    def fwd16():
        for i in range(D // 16):
            rs = slice(i * 16, (i + 1) * 16)
            xs = [u_ref[rs, a * 128:(a + 1) * 128] for a in range(16)]
            ys = _rfft16(xs)
            for b in range(16):
                r_ref[rs, b * 128:(b + 1) * 128] = ys[b].astype(BF16)
            if i % 2 == 1:
                yield

    def filtprep(part, src):
        for a in range(16):
            wa_ref[a, 0:DF, :] = src[:, a * 128:(a + 1) * 128].astype(F32)
            for k0, n, r0 in _RES:
                wb_ref[a, r0:r0 + n, :] = wa_ref[a, pl.ds(k0, n, stride=9), :]
            for t in range(3):
                wc_ref[t, a * 128:(a + 1) * 128, :] = wb_ref[a, t * 128:(t + 1) * 128, :].T
            if a % 2 == 1:
                yield
        frow = jax.lax.broadcasted_iota(jnp.int32, (128, 128), 0)
        edge = jnp.where((frow == 0) | (frow == 32), 1.0, 2.0).astype(F32) * (1.0 / (S * D))
        for k1 in range(16):
            wf_ref[part, k1, 0:128, :] = wc_ref[0, pl.ds(k1, 128, stride=16), :].T * edge
            wf_ref[part, k1, 128:256, :] = wc_ref[1, pl.ds(k1, 128, stride=16), :].T * (2.0 / (S * D))
            wf_ref[part, k1, 256:NR, :] = (wc_ref[2, pl.ds(k1, 128, stride=16), :].T[0:NR - 256]
                                           * (2.0 / (S * D)))
            if k1 % 2 == 1:
                yield

    def interleave(*gens):
        gens = list(gens)
        while gens:
            for g in list(gens):
                try:
                    next(g)
                except StopIteration:
                    gens.remove(g)

    def proj(i):
        mb = HB * DH
        for n in range(PC // 128):
            c0 = i * PC + n * 128
            cs = slice(c0, c0 + 128)
            xc = bx_ref[:, cs]
            for blk in range(3 * D // mb):
                pr = _dot(wt_ref[blk * mb:(blk + 1) * mb, :], xc, _NN)
                part, b = divmod(blk, D // mb)
                if part == 2:
                    for r in range(HB):
                        vt_ref[b * HB + r, 0:DH, cs] = pr[r * DH:(r + 1) * DH, :]
                    yield
                    continue
                for gi, h0 in enumerate(_GS):
                    h1 = (_GS + (HB,))[gi + 1]
                    w = (h1 - h0) * DH
                    g = 3 * b + gi
                    if part == 0:
                        qt_ref[g, 0:w, cs] = pr[h0 * DH:h1 * DH, :] * _QSCALE
                    else:
                        kt_ref[g, 0:w, cs] = pr[h0 * DH:h1 * DH, :]
                        k_ref[g, cs, :] = kt_ref[g, :, cs].astype(BF16).T
                yield

    def fwd_d():
        t0 = _dot(fd_ref[0, 0:80, 0:64], r_ref[0:64, :], _NN)
        t_ref[0, 0:40, :] = t0[0:40]
        t_ref[1, 0:40, :] = t0[40:80]
        for c in range(1, 5):
            tc = _dot(fd_ref[c], r_ref[64 + 128 * (c - 1):64 + 128 * c, :], _NN)
            t_ref[0, 40 + 64 * (c - 1):40 + 64 * c, :] = tc[0:64]
            t_ref[1, 40 + 64 * (c - 1):40 + 64 * c, :] = tc[64:128]
            yield

    cp_bx[0].wait()
    interleave(proj(0))
    cp_bx[1].wait()
    cp_ax.wait()
    cp_wr.wait()
    interleave(proj(1), fwd9(), filtprep(0, wr_ref))
    cp_bx[2].wait()
    cp_wi.wait()
    interleave(proj(2), fwd16(), filtprep(1, wi_ref))
    cp_bx[3].wait()
    cp_fd.wait()
    interleave(proj(3), fwd_d())

    cp_g.wait()

    def spectral(k1, lr, li):
        gm = g_ref[k1]
        y = _dot(jnp.concatenate([lr, li], axis=1).astype(BF16), gm, _NN)
        yr, yi = y[:, :128], y[:, 128:]
        wr = wf_ref[0, k1]
        wi = wf_ref[1, k1]
        z = jnp.concatenate([yr * wr - yi * wi, yr * wi + yi * wr], axis=1).astype(BF16)
        b = _dot(z, gm, _NT)
        return b[:, :128], b[:, 128:]

    def put_u(blk, ur, ui):
        cs = slice(blk * 128, (blk + 1) * 128)
        ub_ref[0:40, cs] = ur[0:40]
        ub_ref[40:80, cs] = ui[0:40]
        for c in range(1, 5):
            ub_ref[128 * c:128 * c + 64, cs] = ur[40 + 64 * (c - 1):40 + 64 * c]
            ub_ref[128 * c + 64:128 * c + 128, cs] = ui[40 + 64 * (c - 1):40 + 64 * c]

    def get_t(blk):
        cs = slice(blk * 128, (blk + 1) * 128)
        return t_ref[0, :, cs], t_ref[1, :, cs]

    def pair(k1):
        drr, dir_ = get_t(2 * k1)
        dri, dii = get_t(2 * k1 + 1)
        br1, bi1 = spectral(k1, drr - dii, dir_ + dri)
        br2, bi2 = spectral(16 - k1, drr + dii, dir_ - dri)
        put_u(2 * k1, br1 + br2, bi1 + bi2)
        put_u(2 * k1 + 1, bi1 - bi2, br2 - br1)

    for p, k1 in ((0, 0), (1, 8)):
        lr, li = get_t(p)
        br, bi = spectral(k1, lr, li)
        put_u(p, br, bi)
    for k1 in range(1, 8):
        pair(k1)

    u_ref[0:64, :] = _dot(fd_ref[5, 0:64, 0:80], ub_ref[0:80, :].astype(BF16), _NN)
    for c in range(1, 5):
        u_ref[64 + 128 * (c - 1):64 + 128 * c, :] = _dot(
            fd_ref[5 + c], ub_ref[128 * c:128 * (c + 1), :].astype(BF16), _NN)

    def inv16():
        for i in range(D // 16):
            rs = slice(i * 16, (i + 1) * 16)
            hs = [u_ref[rs, b * 128:(b + 1) * 128] for b in range(16)]
            ys = _irfft16(hs)
            for a in range(16):
                u_ref[rs, a * 128:(a + 1) * 128] = ys[a]
            if i % 2 == 1:
                yield

    qrows = jax.lax.broadcasted_iota(jnp.int32, (128, TQ), 0)

    def get_q(h, j):
        r = h % HB
        gi = jnp.where(r >= _GS[2], 2, jnp.where(r >= _GS[1], 1, 0))
        g = 3 * (h // HB) + gi
        lo = (r - jnp.where(r >= _GS[2], _GS[2], jnp.where(r >= _GS[1], _GS[1], 0))) * DH
        q = qt_ref[g, :, j * TQ:(j + 1) * TQ]
        q = jnp.where((qrows >= lo) & (qrows < lo + DH), q, 0.0).astype(BF16)
        return g, q

    def stage_a(c, g, q, s_ref, m):
        s = _dot(k_ref[g, c * TK:(c + 1) * TK, :], q, _NN)
        s_ref[c * TK:(c + 1) * TK, :] = s
        return jnp.maximum(m, jnp.max(s.reshape(TK // 8, 8, TQ), axis=0))

    def stage_b(c, h, s_ref, m, acc):
        p = jnp.exp2(s_ref[c * TK:(c + 1) * TK, :] - m)
        return acc + _dot(vt_ref[h, :, c * TK:(c + 1) * TK], p, _NN)

    def prologue():
        g0, q0 = get_q(0, 0)
        mi = jnp.full((8, TQ), -jnp.inf, F32)
        for c in range(NK):
            mi = stage_a(c, g0, q0, s0_ref, mi)
            yield
        m0_ref[...] = jnp.max(mi, axis=0, keepdims=True)

    cp_wo.wait()
    interleave(prologue(), inv16())
    wo32 = wo_ref[...].astype(F32)
    for p in range(H // HPI):
        wop_ref[p * PR + 32:(p + 1) * PR, :] = jnp.zeros((8, D), F32)
        wop_ref[p * PR:p * PR + HPI * DH, :] = wo32[p * HPI * DH:(p + 1) * HPI * DH, :]
    wot_ref[...] = wop_ref[...].astype(BF16).T

    def att_body(i, _):
        for hh in range(HPI):
            h = i * HPI + hh
            for j in range(NQ):
                even = (hh * NQ + j) % 2 == 0
                scur, snext = (s0_ref, s1_ref) if even else (s1_ref, s0_ref)
                mcur_ref, mnext_ref = (m0_ref, m1_ref) if even else (m1_ref, m0_ref)
                mcur = mcur_ref[...]
                if j + 1 < NQ:
                    g, q = get_q(h, j + 1)
                else:
                    g, q = get_q(jnp.minimum(h + 1, H - 1), 0)
                mn = jnp.full((8, TQ), -jnp.inf, F32)
                acc = jnp.zeros((OP, TQ), F32)
                for c in range(NK + SKEW):
                    if c < NK:
                        mn = stage_a(c, g, q, snext, mn)
                    if c == NK - 1:
                        mnext_ref[...] = jnp.max(mn, axis=0, keepdims=True)
                    if c >= SKEW:
                        acc = stage_b(c - SKEW, h, scur, mcur, acc)
                ot_ref[i, hh * DH:(hh + 1) * DH, j * TQ:(j + 1) * TQ] = acc[0:DH] / acc[DH:DH + 1, :]
        return 0

    jax.lax.fori_loop(0, H // HPI, att_body, 0)

    OC = 128
    NOC = S // OC

    def out_copy(i):
        rs = slice(i * OC, (i + 1) * OC)
        return pltpu.make_async_copy(out_ref.at[rs, :], out_hbm.at[rs, :], out_sems.at[i])

    def oproj(i):
        cs = slice(i * OC, (i + 1) * OC)
        o = ot_ref[:, :, cs].reshape(H // HPI * PR, OC).astype(BF16)
        ob = _dot(wot_ref[...], o, _NN)
        out_ref[cs, D:2 * D] = ob.astype(BF16).T
        for q in range(4):
            for n in range(OC // 128):
                c1 = slice(i * OC + n * 128, i * OC + (n + 1) * 128)
                hs = [u_ref[a * 64 + q * 16:a * 64 + (q + 1) * 16, c1] for a in range(9)]
                ys = _irfft9(hs)
                for a in range(9):
                    r_ref[a * 64 + q * 16:a * 64 + (q + 1) * 16, c1] = ys[a].astype(BF16)
        out_ref[cs, 0:D] = r_ref[:, cs].T

    for i in range(NOC):
        oproj(i)
        if i > 0:
            out_copy(i - 1).start()
    out_copy(NOC - 1).start()
    for i in range(NOC):
        out_copy(i).wait()


@jax.jit
def pallas_concat_heads__spectral_gfnet__mha_block__prompt_kernel(
    A_x: jax.Array,
    A_w_r: jax.Array,
    A_w_i: jax.Array,
    B_x: jax.Array,
    B_wqkv: jax.Array,
    B_wo: jax.Array,
):
    fd = jnp.asarray(_FD_NP, dtype=BF16)
    gm = jnp.asarray(_G_NP, dtype=BF16)
    hbm_spec = pl.BlockSpec(memory_space=pltpu.HBM)
    vm = pltpu.VMEM
    out = pl.pallas_call(
        _kernel,
        in_specs=[hbm_spec] * 8,
        out_specs=hbm_spec,
        out_shape=jax.ShapeDtypeStruct((S, 2 * D), BF16),
        scratch_shapes=[
            vm((D, S), BF16), vm((DF, S), BF16), vm((DF, S), BF16), vm((D, S), BF16),
            vm((D, 3 * D), BF16), vm((D, D), BF16), vm((10, 128, 128), BF16), vm((16, 256, 256), BF16),
            vm((S, 2 * D), BF16),
            vm((3 * D, D), BF16),
            vm((D, H // HPI * PR), BF16),
            vm((NG, S, 128), BF16),
            vm((NG, 128, S), F32),
            vm((NG, 128, S), F32),
            vm((H, OP, S), F32),
            vm((H // HPI, PR, S), F32),
            vm((H // HPI * PR, D), F32),
            vm((S, TQ), F32), vm((S, TQ), F32), vm((1, TQ), F32), vm((1, TQ), F32),
            vm((D, S), F32),
            vm((D, S), BF16),
            vm((2, NR, S), F32),
            vm((640, S), F32),
            vm((16, NR + 8, 128), F32), vm((16, 384, 128), F32), vm((3, S + 16, 128), F32),
            vm((2, 16, NR, 128), F32),
            pltpu.SemaphoreType.DMA((13,)),
            pltpu.SemaphoreType.DMA((S // 128,)),
        ],
        compiler_params=pltpu.CompilerParams(vmem_limit_bytes=110 * 2 ** 20),
    )(A_x.reshape(S, D).T, A_w_r.T, A_w_i.T, B_x.reshape(S, D).T, B_wqkv, B_wo, fd, gm)
    return out.reshape(1, S, 2 * D)
```

```python
import math

import numpy as np
import jax
import jax.numpy as jnp
import jax.experimental.pallas as pl
import jax.experimental.pallas.tpu as pltpu

S = 2048
D = 576
H = 32
DH = 18
DF = D // 2 + 1
NR = 296
HB = 16
_GS = (0, 6, 11)
NG = 6
TQ = 512
TK = 128
SKEW = 2
HPI = 2
PR = 40
NQ = S // TQ
NK = S // TK
OP = 24
F32 = jnp.float32
BF16 = jnp.bfloat16

_C1 = math.cos(math.pi / 8)
_C3 = math.cos(3 * math.pi / 8)
_R2 = math.cos(math.pi / 4)
_N1, _N2, _N4 = (math.cos(2 * math.pi * k / 9) for k in (1, 2, 4))
_S1, _S3, _S4 = (math.sin(2 * math.pi * k / 9) for k in (1, 3, 4))


def _dft_constants():
    b = np.arange(64)[None, :]
    f0 = np.zeros((128, 128))
    j = np.arange(33)[:, None]
    th = 2 * np.pi * ((b * 9 * j) % D) / D
    f0[:33, :64] = np.cos(th)
    f0[40:73, :64] = -np.sin(th)
    fc = np.zeros((5, 128, 128))
    fc[0] = f0
    j = np.arange(32)[:, None]
    for c in range(1, 5):
        th = 2 * np.pi * ((b * (c + 9 * j)) % D) / D
        th2 = 2 * np.pi * ((b * (9 - c + 9 * j)) % D) / D
        fc[c, 0:32] = np.concatenate([np.cos(th), np.sin(th)], 1)
        fc[c, 32:64] = np.concatenate([np.cos(th2), -np.sin(th2)], 1)
        fc[c, 64:96] = np.concatenate([-np.sin(th), np.cos(th)], 1)
        fc[c, 96:128] = np.concatenate([-np.sin(th2), -np.cos(th2)], 1)
    fd = np.concatenate([fc, fc.transpose(0, 2, 1)], 0)
    n2 = np.arange(128)[:, None]
    j = np.arange(128)[None, :]
    g = np.zeros((16, 256, 256))
    for k1 in range(16):
        a = -2 * np.pi * ((n2 * (k1 + 16 * j)) % S) / S
        cr, ci = np.cos(a), np.sin(a)
        g[k1] = np.block([[cr, ci], [-ci, cr]])
    return fd.astype(np.float32), g.astype(np.float32)


_FD_NP, _G_NP = _dft_constants()
_QSCALE = float(np.asarray(DH ** -0.5, np.float32).astype(jnp.bfloat16).astype(np.float32)) * math.log2(math.e)
_RES = [(0, 33, 0)] + [r for c in range(1, 5)
                       for r in ((c, 32, 40 + 64 * (c - 1)), (9 - c, 32, 72 + 64 * (c - 1)))]


def _rfft16(x):
    a = [x[n] + x[n + 8] for n in range(8)]
    b = [x[n] - x[n + 8] for n in range(8)]
    c = [a[n] + a[n + 4] for n in range(4)]
    d = [a[n] - a[n + 4] for n in range(4)]
    s02, s13 = c[0] + c[2], c[1] + c[3]
    x0, x8 = s02 + s13, s02 - s13
    x4r, x4i = c[0] - c[2], c[3] - c[1]
    t1 = (d[1] - d[3]) * _R2
    t2 = (d[1] + d[3]) * _R2
    x2r, x6r = d[0] + t1, d[0] - t1
    x2i, x6i = -(d[2] + t2), d[2] - t2
    e = {n: b[n] - b[8 - n] for n in (1, 2, 3)}
    f = {n: b[n] + b[8 - n] for n in (1, 2, 3)}
    re2 = e[2] * _R2
    u, v = b[0] + re2, b[0] - re2
    p = e[1] * _C1 + e[3] * _C3
    s = e[1] * _C3 - e[3] * _C1
    x1r, x7r, x3r, x5r = u + p, u - p, v + s, v - s
    g = f[2] * _R2
    pp = f[1] * _C3 + f[3] * _C1
    qq = f[1] * _C1 - f[3] * _C3
    g1, g2 = g + b[4], g - b[4]
    x1i, x7i = -(pp + g1), g1 - pp
    x3i, x5i = -(qq + g2), g2 - qq
    return [x0, x8, x1r, x1i, x2r, x2i, x3r, x3i, x4r, x4i, x5r, x5i, x6r, x6i, x7r, x7i]


def _irfft16(h):
    h0, h8, h1r, h1i, h2r, h2i, h3r, h3i, h4r, h4i, h5r, h5i, h6r, h6i, h7r, h7i = h
    u, pp = h1r + h7r, h1r - h7r
    v, ss = h3r + h5r, h3r - h5r
    b0 = u + v
    e2 = (u - v) * _R2
    e1 = pp * _C1 + ss * _C3
    e3 = pp * _C3 - ss * _C1
    p1, g1 = -(h1i + h7i), h7i - h1i
    q1, g2 = -(h3i + h5i), h5i - h3i
    b4 = g1 - g2
    f2 = (g1 + g2) * _R2
    f1 = p1 * _C3 + q1 * _C1
    f3 = p1 * _C1 - q1 * _C3
    b = [b0, e1 + f1, e2 + f2, e3 + f3, b4, f3 - e3, f2 - e2, f1 - e1]
    d0 = h2r + h6r
    t1 = (h2r - h6r) * _R2
    d2 = h6i - h2i
    t2 = (h2i + h6i) * (-_R2)
    d = [d0, t1 + t2, d2, t2 - t1]
    s02, s13 = h0 + h8, h0 - h8
    c = [s02 + h4r, s13 - h4i, s02 - h4r, s13 + h4i]
    a = [c[n] + d[n] for n in range(4)] + [c[n] - d[n] for n in range(4)]
    return [a[n] + b[n] for n in range(8)] + [a[n] - b[n] for n in range(8)]


def _rfft9(x):
    s1, s2, s3, s4 = [x[a] + x[9 - a] for a in (1, 2, 3, 4)]
    d1, d2, d3, d4 = [x[a] - x[9 - a] for a in (1, 2, 3, 4)]
    t = x[0] - 0.5 * s3
    u = s1 + s2 + s4
    z = x[0] + s3
    a0 = z + u
    ar3 = z - 0.5 * u
    p, q = s1 - s4, s2 - s4
    ar1 = t + (_N1 * p + _N2 * q)
    ar2 = t + (_N2 * p + _N4 * q)
    ar4 = t + (_N4 * p + _N1 * q)
    e, f, g = d1 + d2, d2 + d4, d1 - d4
    w = _S3 * d3
    ai1 = ((-_S1) * e - _S4 * f) - w
    ai2 = w - (_S1 * g + _S4 * e)
    ai4 = (_S1 * f - _S4 * g) - w
    ai3 = (d2 - d1 - d4) * _S3
    return [a0, ar1, ai1, ar2, ai2, ar3, ai3, ar4, ai4]


def _irfft9(h):
    h0, hr1, hi1, hr2, hi2, hr3, hi3, hr4, hi4 = h
    t = hr1 + hr2 + hr4
    p = _N1 * (hr1 - hr4) + _N2 * (hr2 - hr4)
    q = _N2 * (hr1 - hr2) + _N1 * (hr4 - hr2)
    z = h0 + hr3
    u = h0 - 0.5 * hr3
    x0 = z + t
    s3 = z - 0.5 * t
    s1, s2, s4 = u + p, u + q, u - p - q
    e = (-_S1) * hi1 - _S4 * hi2
    f = _S1 * hi4 - _S4 * hi1
    g = (-_S1) * hi2 - _S4 * hi4
    d3 = (hi2 - hi1 - hi4) * _S3
    v = (-_S3) * hi3
    d1, d2, d4 = e + g + v, e + f - v, f - g + v
    return [x0, s1 + d1, s2 + d2, s3 + d3, s4 + d4, s4 - d4, s3 - d3, s2 - d2, s1 - d1]


def _dot(a, b, dims):
    return jax.lax.dot_general(a, b, (dims, ((), ())), preferred_element_type=F32)


_NN = ((1,), (0,))
_NT = ((1,), (1,))


def _kernel(ax_hbm, wr_hbm, wi_hbm, bx_hbm, wqkv_hbm, wo_hbm, fd_hbm, g_hbm,
            out_hbm,
            ax_ref, wr_ref, wi_ref, bx_ref, wqkv_ref, wo_ref, fd_ref, g_ref,
            out_ref, wt_ref, wot_ref, k_ref, kt_ref, qt_ref, vt_ref, ot_ref, wop_ref,
            s0_ref, s1_ref, m0_ref, m1_ref,
            u_ref, r_ref, t_ref, ub_ref, wa_ref, wb_ref, wc_ref, wf_ref,
            in_sems, out_sems):
    PC = 512
    NPC = S // PC
    wcs = [slice(c, min(c + 384, 3 * D)) for c in range(0, 3 * D, 384)]
    NW = len(wcs)
    cp_w = [pltpu.make_async_copy(wqkv_hbm.at[:, cs], wqkv_ref.at[:, cs], in_sems.at[t])
            for t, cs in enumerate(wcs)]
    cp_bx = [pltpu.make_async_copy(bx_hbm.at[:, i * PC:(i + 1) * PC], bx_ref.at[:, i * PC:(i + 1) * PC],
                                   in_sems.at[NW + i]) for i in range(NPC)]
    srcs = (ax_hbm, wr_hbm, wi_hbm, fd_hbm, g_hbm, wo_hbm)
    dsts = (ax_ref, wr_ref, wi_ref, fd_ref, g_ref, wo_ref)
    rest = [pltpu.make_async_copy(s, d, in_sems.at[NW + NPC + i]) for i, (s, d) in enumerate(zip(srcs, dsts))]
    cp_ax, cp_wr, cp_wi, cp_fd, cp_g, cp_wo = rest
    for cp in cp_w[:1] + cp_bx[:1] + cp_w[1:] + cp_bx[1:2] + rest[:3] + cp_bx[2:] + rest[3:]:
        cp.start()

    gws = [((_GS + (HB,))[gi + 1] - h0) * DH for gi, h0 in enumerate(_GS)]
    for g in range(NG):
        lo8 = gws[g % 3] // 8 * 8
        kt_ref[g, lo8:128, :] = jnp.zeros((128 - lo8, S), F32)

    def consts():
        for g in range(NG):
            lo8 = gws[g % 3] // 8 * 8
            qt_ref[g, lo8:128, :] = jnp.zeros((128 - lo8, S), F32)
        rows8 = jax.lax.broadcasted_iota(jnp.int32, (8, S), 0)
        tail = jnp.where(rows8 == DH - 16, 1.0, 0.0).astype(F32)
        for h in range(H):
            vt_ref[h, 16:OP, :] = tail
        ot_ref[:, 32:PR, :] = jnp.zeros((H // HPI, 8, S), F32)
        wb_ref[:, 32:40, :] = jnp.zeros((16, 8, 128), F32)
        wb_ref[:, NR:384, :] = jnp.zeros((16, 384 - NR, 128), F32)

    consts()

    def fwd9():
        for i in range(4):
            for qd in range(16):
                cs = slice(qd * 128, (qd + 1) * 128)
                xs = [ax_ref[a * 64 + i * 16:a * 64 + (i + 1) * 16, cs].astype(F32) for a in range(9)]
                ys = _rfft9(xs)
                for a in range(9):
                    u_ref[a * 64 + i * 16:a * 64 + (i + 1) * 16, cs] = ys[a]
                if qd % 4 == 3:
                    yield

    def fwd16():
        for i in range(D // 16):
            rs = slice(i * 16, (i + 1) * 16)
            xs = [u_ref[rs, a * 128:(a + 1) * 128] for a in range(16)]
            ys = _rfft16(xs)
            for b in range(16):
                r_ref[rs, b * 128:(b + 1) * 128] = ys[b].astype(BF16)
            if i % 2 == 1:
                yield

    def filtprep(part, src):
        for a in range(16):
            wa_ref[a, 0:DF, :] = src[:, a * 128:(a + 1) * 128].astype(F32)
            for k0, n, r0 in _RES:
                wb_ref[a, r0:r0 + n, :] = wa_ref[a, pl.ds(k0, n, stride=9), :]
            for t in range(3):
                wc_ref[t, a * 128:(a + 1) * 128, :] = wb_ref[a, t * 128:(t + 1) * 128, :].T
            if a % 2 == 1:
                yield
        frow = jax.lax.broadcasted_iota(jnp.int32, (128, 128), 0)
        edge = jnp.where((frow == 0) | (frow == 32), 1.0, 2.0).astype(F32) * (1.0 / (S * D))
        for k1 in range(16):
            wf_ref[part, k1, 0:128, :] = wc_ref[0, pl.ds(k1, 128, stride=16), :].T * edge
            wf_ref[part, k1, 128:256, :] = wc_ref[1, pl.ds(k1, 128, stride=16), :].T * (2.0 / (S * D))
            wf_ref[part, k1, 256:NR, :] = (wc_ref[2, pl.ds(k1, 128, stride=16), :].T[0:NR - 256]
                                           * (2.0 / (S * D)))
            if k1 % 2 == 1:
                yield

    def interleave(*gens):
        gens = list(gens)
        while gens:
            for g in list(gens):
                try:
                    next(g)
                except StopIteration:
                    gens.remove(g)

    MB = HB * DH

    def proj(i, blks=tuple(range(3 * D // MB))):
        for blk in blks:
            for n in range(PC // 128):
                c0 = i * PC + n * 128
                cs = slice(c0, c0 + 128)
                pr = _dot(wt_ref[blk * MB:(blk + 1) * MB, :], bx_ref[:, cs], _NN)
                part, b = divmod(blk, D // MB)
                if part == 2:
                    for r in range(HB):
                        vt_ref[b * HB + r, 0:DH, cs] = pr[r * DH:(r + 1) * DH, :]
                    yield
                    continue
                for gi, h0 in enumerate(_GS):
                    h1 = (_GS + (HB,))[gi + 1]
                    w = (h1 - h0) * DH
                    g = 3 * b + gi
                    if part == 0:
                        qt_ref[g, 0:w, cs] = pr[h0 * DH:h1 * DH, :] * _QSCALE
                    else:
                        kt_ref[g, 0:w, cs] = pr[h0 * DH:h1 * DH, :]
                        k_ref[g, cs, :] = kt_ref[g, :, cs].astype(BF16).T
                yield

    def fwd_d():
        t0 = _dot(fd_ref[0, 0:80, 0:64], r_ref[0:64, :], _NN)
        t_ref[0, 0:40, :] = t0[0:40]
        t_ref[1, 0:40, :] = t0[40:80]
        for c in range(1, 5):
            tc = _dot(fd_ref[c], r_ref[64 + 128 * (c - 1):64 + 128 * c, :], _NN)
            t_ref[0, 40 + 64 * (c - 1):40 + 64 * c, :] = tc[0:64]
            t_ref[1, 40 + 64 * (c - 1):40 + 64 * c, :] = tc[64:128]
            yield

    done = 0
    for t, cs in enumerate(wcs):
        cp_w[t].wait()
        wt_ref[cs, :] = wqkv_ref[:, cs].T
        if t == 0:
            cp_bx[0].wait()
        ready = cs.stop // MB
        interleave(proj(0, tuple(range(done, ready))))
        done = ready
    cp_bx[1].wait()
    cp_ax.wait()
    cp_wr.wait()
    interleave(proj(1), fwd9(), filtprep(0, wr_ref))
    cp_bx[2].wait()
    cp_wi.wait()
    interleave(proj(2), fwd16(), filtprep(1, wi_ref))
    cp_bx[3].wait()
    cp_fd.wait()
    interleave(proj(3), fwd_d())

    cp_g.wait()

    def spectral(k1, lr, li):
        gm = g_ref[k1]
        y = _dot(jnp.concatenate([lr, li], axis=1).astype(BF16), gm, _NN)
        yr, yi = y[:, :128], y[:, 128:]
        wr = wf_ref[0, k1]
        wi = wf_ref[1, k1]
        z = jnp.concatenate([yr * wr - yi * wi, yr * wi + yi * wr], axis=1).astype(BF16)
        b = _dot(z, gm, _NT)
        return b[:, :128], b[:, 128:]

    def put_u(blk, ur, ui):
        cs = slice(blk * 128, (blk + 1) * 128)
        ub_ref[0:40, cs] = ur[0:40]
        ub_ref[40:80, cs] = ui[0:40]
        for c in range(1, 5):
            ub_ref[128 * c:128 * c + 64, cs] = ur[40 + 64 * (c - 1):40 + 64 * c]
            ub_ref[128 * c + 64:128 * c + 128, cs] = ui[40 + 64 * (c - 1):40 + 64 * c]

    def get_t(blk):
        cs = slice(blk * 128, (blk + 1) * 128)
        return t_ref[0, :, cs], t_ref[1, :, cs]

    def pair(k1):
        drr, dir_ = get_t(2 * k1)
        dri, dii = get_t(2 * k1 + 1)
        br1, bi1 = spectral(k1, drr - dii, dir_ + dri)
        br2, bi2 = spectral(16 - k1, drr + dii, dir_ - dri)
        put_u(2 * k1, br1 + br2, bi1 + bi2)
        put_u(2 * k1 + 1, bi1 - bi2, br2 - br1)

    for p, k1 in ((0, 0), (1, 8)):
        lr, li = get_t(p)
        br, bi = spectral(k1, lr, li)
        put_u(p, br, bi)
    for k1 in range(1, 8):
        pair(k1)

    u_ref[0:64, :] = _dot(fd_ref[5, 0:64, 0:80], ub_ref[0:80, :].astype(BF16), _NN)
    for c in range(1, 5):
        u_ref[64 + 128 * (c - 1):64 + 128 * c, :] = _dot(
            fd_ref[5 + c], ub_ref[128 * c:128 * (c + 1), :].astype(BF16), _NN)

    def inv16():
        for i in range(D // 16):
            rs = slice(i * 16, (i + 1) * 16)
            hs = [u_ref[rs, b * 128:(b + 1) * 128] for b in range(16)]
            ys = _irfft16(hs)
            for a in range(16):
                u_ref[rs, a * 128:(a + 1) * 128] = ys[a]
            if i % 2 == 1:
                yield

    qrows = jax.lax.broadcasted_iota(jnp.int32, (128, TQ), 0)

    def get_q(h, j):
        r = h % HB
        gi = jnp.where(r >= _GS[2], 2, jnp.where(r >= _GS[1], 1, 0))
        g = 3 * (h // HB) + gi
        lo = (r - jnp.where(r >= _GS[2], _GS[2], jnp.where(r >= _GS[1], _GS[1], 0))) * DH
        q = qt_ref[g, :, j * TQ:(j + 1) * TQ]
        q = jnp.where((qrows >= lo) & (qrows < lo + DH), q, 0.0).astype(BF16)
        return g, q

    def stage_a(c, g, q, s_ref, m):
        s = _dot(k_ref[g, c * TK:(c + 1) * TK, :], q, _NN)
        s_ref[c * TK:(c + 1) * TK, :] = s
        return jnp.maximum(m, jnp.max(s.reshape(TK // 8, 8, TQ), axis=0))

    def stage_b(c, h, s_ref, m, acc):
        p = jnp.exp2(s_ref[c * TK:(c + 1) * TK, :] - m)
        return acc + _dot(vt_ref[h, :, c * TK:(c + 1) * TK], p, _NN)

    def prologue():
        g0, q0 = get_q(0, 0)
        mi = jnp.full((8, TQ), -jnp.inf, F32)
        for c in range(NK):
            mi = stage_a(c, g0, q0, s0_ref, mi)
            yield
        m0_ref[...] = jnp.max(mi, axis=0, keepdims=True)

    cp_wo.wait()
    interleave(prologue(), inv16())
    wo32 = wo_ref[...].astype(F32)
    for p in range(H // HPI):
        wop_ref[p * PR + 32:(p + 1) * PR, :] = jnp.zeros((8, D), F32)
        wop_ref[p * PR:p * PR + HPI * DH, :] = wo32[p * HPI * DH:(p + 1) * HPI * DH, :]
    wot_ref[...] = wop_ref[...].astype(BF16).T

    def att_body(i, _, last=False):
        for hh in range(HPI):
            h = i * HPI + hh
            for j in range(NQ):
                even = (hh * NQ + j) % 2 == 0
                scur, snext = (s0_ref, s1_ref) if even else (s1_ref, s0_ref)
                mcur_ref, mnext_ref = (m0_ref, m1_ref) if even else (m1_ref, m0_ref)
                mcur = mcur_ref[...]
                has_next = not (last and hh == HPI - 1 and j == NQ - 1)
                if has_next:
                    g, q = get_q(h, j + 1) if j + 1 < NQ else get_q(h + 1, 0)
                mn = jnp.full((8, TQ), -jnp.inf, F32)
                acc = jnp.zeros((OP, TQ), F32)
                for c in range(NK + SKEW):
                    if c < NK and has_next:
                        mn = stage_a(c, g, q, snext, mn)
                    if c == NK - 1 and has_next:
                        mnext_ref[...] = jnp.max(mn, axis=0, keepdims=True)
                    if c >= SKEW:
                        acc = stage_b(c - SKEW, h, scur, mcur, acc)
                ot_ref[i, hh * DH:(hh + 1) * DH, j * TQ:(j + 1) * TQ] = acc[0:DH] / acc[DH:DH + 1, :]
        return 0

    att_body(0, 0)
    jax.lax.fori_loop(1, H // HPI - 1, att_body, 0)
    att_body(H // HPI - 1, 0, last=True)

    OC = 128
    NOC = S // OC

    def out_copy(i):
        rs = slice(i * OC, (i + 1) * OC)
        return pltpu.make_async_copy(out_ref.at[rs, :], out_hbm.at[rs, :], out_sems.at[i])

    def oproj(i):
        cs = slice(i * OC, (i + 1) * OC)
        o = ot_ref[:, :, cs].reshape(H // HPI * PR, OC).astype(BF16)
        ob = _dot(wot_ref[...], o, _NN)
        out_ref[cs, D:2 * D] = ob.astype(BF16).T
        for q in range(4):
            for n in range(OC // 128):
                c1 = slice(i * OC + n * 128, i * OC + (n + 1) * 128)
                hs = [u_ref[a * 64 + q * 16:a * 64 + (q + 1) * 16, c1] for a in range(9)]
                ys = _irfft9(hs)
                for a in range(9):
                    r_ref[a * 64 + q * 16:a * 64 + (q + 1) * 16, c1] = ys[a].astype(BF16)
        out_ref[cs, 0:D] = r_ref[:, cs].T

    for i in range(NOC):
        oproj(i)
        if i > 0:
            out_copy(i - 1).start()
    out_copy(NOC - 1).start()
    for i in range(NOC):
        out_copy(i).wait()


@jax.jit
def pallas_concat_heads__spectral_gfnet__mha_block__prompt_kernel(
    A_x: jax.Array,
    A_w_r: jax.Array,
    A_w_i: jax.Array,
    B_x: jax.Array,
    B_wqkv: jax.Array,
    B_wo: jax.Array,
):
    fd = jnp.asarray(_FD_NP, dtype=BF16)
    gm = jnp.asarray(_G_NP, dtype=BF16)
    hbm_spec = pl.BlockSpec(memory_space=pltpu.HBM)
    vm = pltpu.VMEM
    out = pl.pallas_call(
        _kernel,
        in_specs=[hbm_spec] * 8,
        out_specs=hbm_spec,
        out_shape=jax.ShapeDtypeStruct((S, 2 * D), BF16),
        scratch_shapes=[
            vm((D, S), BF16), vm((DF, S), BF16), vm((DF, S), BF16), vm((D, S), BF16),
            vm((D, 3 * D), BF16), vm((D, D), BF16), vm((10, 128, 128), BF16), vm((16, 256, 256), BF16),
            vm((S, 2 * D), BF16),
            vm((3 * D, D), BF16),
            vm((D, H // HPI * PR), BF16),
            vm((NG, S, 128), BF16),
            vm((NG, 128, S), F32),
            vm((NG, 128, S), F32),
            vm((H, OP, S), F32),
            vm((H // HPI, PR, S), F32),
            vm((H // HPI * PR, D), F32),
            vm((S, TQ), F32), vm((S, TQ), F32), vm((1, TQ), F32), vm((1, TQ), F32),
            vm((D, S), F32),
            vm((D, S), BF16),
            vm((2, NR, S), F32),
            vm((640, S), F32),
            vm((16, NR + 8, 128), F32), vm((16, 384, 128), F32), vm((3, S + 16, 128), F32),
            vm((2, 16, NR, 128), F32),
            pltpu.SemaphoreType.DMA((15,)),
            pltpu.SemaphoreType.DMA((S // 128,)),
        ],
        compiler_params=pltpu.CompilerParams(vmem_limit_bytes=110 * 2 ** 20),
    )(A_x.reshape(S, D).T, A_w_r.T, A_w_i.T, B_x.reshape(S, D).T, B_wqkv, B_wo, fd, gm)
    return out.reshape(1, S, 2 * D)
```
